```python
import os as _os
_os.environ.setdefault("JAX_PLATFORMS", "cpu")
import jax
import jax.numpy as jnp

def _softmax(x, axis=-1):
    return jax.nn.softmax(x, axis=axis)
def _gelu(x):
    return jax.nn.gelu(x, approximate=True)
def _silu(x):
    return jax.nn.silu(x)
def _sigmoid(x):
    return jax.nn.sigmoid(x)
def _layernorm(x, axis=-1, eps=1e-5):
    m = jnp.mean(x, axis=axis, keepdims=True)
    v = jnp.var(x, axis=axis, keepdims=True)
    return (x - m) / jnp.sqrt(v + eps)
def _scatter_add(tgt, idx, src, axis=0):
    return tgt.at[idx].add(src)
def _segment_sum(src, seg, n):
    return jax.ops.segment_sum(src, seg, n)
class _Rng:
    def __init__(self, key):
        self._k = key
    def _next(self):
        self._k, sub = jax.random.split(self._k)
        return sub
    def normal(self, shape):
        return jax.random.normal(self._next(), shape, dtype=jnp.bfloat16)
    def randint(self, lo, hi, shape):
        return jax.random.randint(self._next(), shape, lo, hi, dtype=jnp.int32)
    def uniform(self, shape, lo=0.0, hi=1.0):
        return jax.random.uniform(self._next(), shape, jnp.bfloat16, lo, hi)
    def permutation(self, n):
        return jax.random.permutation(self._next(), n)


kernel_name = 'sequential_preLN__linear_kernel_hedgehog__dense_activation_squared_relu__prompt'

def setup_inputs():
    _rng = _Rng(jax.random.key(int.from_bytes(__import__("os").urandom(4), "little")))
    _w = (lambda a: (lambda t: t.astype(jnp.bfloat16) if jnp.issubdtype(t.dtype, jnp.floating) else t)(jnp.asarray(a)))
    def _A_setup():
        B, S, D, H = 1, 2048, 512, 32
        Dh = D // H
        return {
            "x": _w((lambda *s: _rng.normal(s) * 0.05)(B, S, D)),
            "wqkv": _w((lambda *s: _rng.normal(s) * 0.2)(D, 3 * D)),
            "w_phi": _w((lambda *s: _rng.normal(s) * 0.2)(H, Dh, Dh) * (Dh ** -0.5)),
            "wo": _w((lambda *s: _rng.normal(s) * 0.05)(D, D)),
        }
    _A_in = _A_setup()

    def _B_setup():
        B, S, D, F = 1, 2048, 512, 1792
        return {
            "x": _w((lambda *s: _rng.normal(s) * 0.05)(B, S, D)),
            "w1": _w((lambda *s: _rng.normal(s) * 0.05)(D, F)),
            "b1": _w((lambda *s: _rng.normal(s) * 0.05)(F)),
            "w2": _w((lambda *s: _rng.normal(s) * 0.05)(F, D)),
            "b2": _w((lambda *s: _rng.normal(s) * 0.05)(D)),
        }
    _B_in = _B_setup()

    return {
        "A_x": _A_in["x"],
        "A_wqkv": _A_in["wqkv"],
        "A_w_phi": _A_in["w_phi"],
        "A_wo": _A_in["wo"],
        "B_x": _B_in["x"],
        "B_w1": _B_in["w1"],
        "B_b1": _B_in["b1"],
        "B_w2": _B_in["w2"],
        "B_b2": _B_in["b2"],
    }

def reference(A_x, A_wqkv, A_w_phi, A_wo, B_x, B_w1, B_b1, B_w2, B_b2):
    def _A_ref(x, wqkv, w_phi, wo):
        B, S, D = x.shape
        H = 32; Dh = D // H
        qkv = (lambda x, *d: x.transpose(*d))((x @ wqkv).reshape(B, S, 3, H, Dh), 2, 0, 3, 1, 4)
        q, k, v = qkv[0], qkv[1], qkv[2]
        pq = jnp.einsum("bhsd,hdf->bhsf", q, w_phi)
        pk = jnp.einsum("bhsd,hdf->bhsf", k, w_phi)
        phi_q = jnp.concatenate([_softmax(pq, axis=-1), _softmax(-pq, axis=-1)], axis=-1)
        phi_k = jnp.concatenate([_softmax(pk, axis=-1), _softmax(-pk, axis=-1)], axis=-1)
        kv = jnp.einsum("bhsf,bhsd->bhfd", phi_k, v)
        z  = jnp.einsum("bhsf->bhf", phi_k)
        num = jnp.einsum("bhqf,bhfd->bhqd", phi_q, kv)
        den = jnp.einsum("bhqf,bhf->bhq", phi_q, z)[..., None] + 1e-6
        o = num / den
        return (lambda x, *d: x.transpose(*d))(o, 0, 2, 1, 3).reshape(B, S, D) @ wo

    def _B_ref(x, w1, b1, w2, b2):
        h = jnp.einsum("bsd,df->bsf", x, w1) + b1
        zero = jnp.zeros_like(h)
        r = jnp.where(h > zero, h, zero)
        h = r * r
        out = jnp.einsum("bsf,fd->bsd", h, w2) + b2
        return out

    x = A_x
    h = x + _A_ref(_layernorm(x, axis=-1), A_wqkv, A_w_phi, A_wo)
    h2 = h + _B_ref(_layernorm(h, axis=-1), B_w1, B_b1, B_w2, B_b2)
    return h2
```

```python
import functools, contextlib
import jax
import jax.numpy as jnp
import numpy as np
import jax.experimental.pallas as pl
import jax.experimental.pallas.tpu as pltpu

S, D, H, DH, F = 2048, 512, 32, 16, 1792
G = 4
HG = 8
LOG2E = float(np.log2(np.e))
NT = (((1,), (1,)), ((), ()))
TN = (((0,), (0,)), ((), ()))
f32, bf16 = jnp.float32, jnp.bfloat16


def _ln(x, onepass):
    m = jnp.sum(x, axis=-1, keepdims=True) * (1.0 / D)
    if onepass:
        v = jnp.maximum(jnp.sum(x * x, axis=-1, keepdims=True) * (1.0 / D) - m * m, 0.0)
        return (x - m) * jax.lax.rsqrt(v + 1e-5)
    d = x - m
    v = jnp.sum(d * d, axis=-1, keepdims=True) * (1.0 / D)
    return d * jax.lax.rsqrt(v + 1e-5)


def _dual_softmax_hg(p):
    n = p.shape[-1]
    p3 = p.reshape(8, 8, n)

    def red(op, fn, a):
        m = fn(a, axis=0)
        m = op(m, pltpu.roll(m, 4, axis=0))
        return m[None]
    mx = red(jnp.maximum, jnp.max, p3)
    mn = red(jnp.minimum, jnp.min, p3)
    ep = jnp.exp2(p3 - mx)
    en = jnp.exp2(mn - p3)
    rp = 1.0 / red(jnp.add, jnp.sum, ep)
    rn = 1.0 / red(jnp.add, jnp.sum, en)
    pp = (ep * rp).reshape(64, n)
    pn = (en * rn).reshape(64, n)
    return jnp.concatenate([pp, pn], axis=0).astype(bf16)


def make_kernel(C2, RB, scopes, tail_split, SB, MR, order, dma, lnpos, unroll2, unr):
    CA, C1 = 256, 512
    n1 = S // C1
    n2 = S // C2

    def scope(name):
        return jax.named_scope(name) if scopes else contextlib.nullcontext()

    def kernel(x_hbm, wqkv_hbm, wphi_hbm, wo_hbm, w1_hbm, b1_hbm, w2_hbm, b2_hbm,
               out_hbm, wphi_ref, b1_ref, b2_ref, rt_v, cs_v,
               x_v, wqkv_v, wt_v, wo_v, wop_v, w1_v, w2_v, acc_v, kvz_v, out_v, h_v, hn_v,
               phik_v, v_v, phiq_v, ot_v,
               sem_x, sem_w, sem_o):
        def rows(start, n):
            return pl.ds(pl.multiple_of(start, min(n, 256)), n)

        def rows2(ci, off=0, n=C2):
            return pl.ds(pl.multiple_of(ci * C2 + off, n), n)

        def wcopy(part, i):
            return pltpu.make_async_copy(wqkv_hbm.at[:, pl.ds(part * D, D)], wqkv_v.at[part], sem_w.at[i])

        def xcopy(c):
            if c < 2:
                r_ = rows(c * CA, CA)
            else:
                r_ = pl.ds(C1, S - C1)
            return pltpu.make_async_copy(x_hbm.at[r_], x_v.at[r_], sem_x.at[c])
        cp = dict(wk=wcopy(1, 0), wv=wcopy(2, 1), wq=wcopy(0, 2),
                  wo=pltpu.make_async_copy(wo_hbm, wo_v, sem_w.at[3]),
                  w1=pltpu.make_async_copy(w1_hbm, w1_v, sem_w.at[4]),
                  w2=pltpu.make_async_copy(w2_hbm, w2_v, sem_w.at[5]),
                  wp=pltpu.make_async_copy(wphi_hbm, wphi_ref, sem_w.at[6]),
                  b1=pltpu.make_async_copy(b1_hbm, b1_ref, sem_w.at[7]),
                  b2=pltpu.make_async_copy(b2_hbm, b2_ref, sem_w.at[8]))
        for c in range(3):
            cp['x%d' % c] = xcopy(c)

        def issue(stage):
            for name in dma.get(stage, ()):
                cp[name].start()
        issue(0)

        with scope("s00_pbuild"):
            cp['wp'].wait()
            issue(20)
            r = jax.lax.broadcasted_iota(jnp.int32, (128, 128), 0)
            c = jax.lax.broadcasted_iota(jnp.int32, (128, 128), 1)
            rj, rh = (r % 64) // 4, (r // 64) * 4 + r % 4
            same_head = rh == (c // 16)
            perm = jnp.where(same_head & ((c % 16) == rj), 1.0, 0.0).astype(bf16)
            z = wphi_ref[...]
            er = jax.lax.broadcasted_iota(jnp.int32, (H, D), 0)
            ec = jax.lax.broadcasted_iota(jnp.int32, (H, D), 1)
            e = jnp.where(er == ec // 16, 1.0, 0.0).astype(bf16)
            ar = jax.lax.broadcasted_iota(jnp.int32, (256, D), 0)
            ac = jax.lax.broadcasted_iota(jnp.int32, (256, D), 1)
            a = jnp.where(ar // 16 == ac % 16, jnp.dot(z, e, preferred_element_type=f32), 0.0).astype(bf16)
            br = jax.lax.broadcasted_iota(jnp.int32, (128, 256), 0)
            bc = jax.lax.broadcasted_iota(jnp.int32, (128, 256), 1)
            r3 = jnp.where((br % 64) // 4 == bc % 16, 1.0, 0.0).astype(bf16)
            pts = []
            for g in range(G):
                t = jnp.dot(r3, a[:, g * 128:(g + 1) * 128], preferred_element_type=f32)
                pts.append(jnp.where(same_head, t, 0.0).astype(bf16))

        def prep(part, mats, scale):
            for g in range(G):
                w = wqkv_v[part, :, pl.ds(g * 128, 128)]
                t = jax.lax.dot_general(mats[g], w, NT, preferred_element_type=f32)
                cs = jnp.sum(t, axis=1, keepdims=True)
                if scale is not None:
                    t = (t - cs * (1.0 / D)) * scale
                else:
                    cs_v[pl.ds(g * 128, 128), :] = jnp.broadcast_to(cs, (128, 128))
                wt_v[pl.ds(part * D + g * 128, 128), :] = t.astype(bf16)

        def rstd(start, n, off):
            outs = []
            for b in range(0, n, 128):
                xf = x_v[rows(start + b, 128), :].astype(f32)
                s1 = xf[:, 0:128]
                s2 = s1 * s1
                for t in range(1, D // 128):
                    xt = xf[:, t * 128:(t + 1) * 128]
                    s1 = s1 + xt
                    s2 = s2 + xt * xt
                def red(a):
                    a = jnp.sum(a.T.reshape(16, 8, 128), axis=0)
                    a = a + pltpu.roll(a, 4, axis=0)
                    a = a + pltpu.roll(a, 2, axis=0)
                    return a + pltpu.roll(a, 1, axis=0)
                m = red(s1) * (1.0 / D)
                v = jnp.maximum(red(s2) * (1.0 / D) - m * m, 0.0)
                outs.append((jax.lax.rsqrt(v + 1e-5), m))
            r_ = jnp.concatenate([o[0] for o in outs], axis=1)
            m_ = jnp.concatenate([o[1] for o in outs], axis=1)
            rt_v[:, pl.ds(start, n)] = r_
            ext = jnp.concatenate([jnp.ones((8, n), f32), r_ * m_], axis=0).astype(bf16)
            for g in range(HG):
                v_v[g, 64:80, off:off + n] = ext
            return r_

        def scale_rows(t, r_):
            n = t.shape[1]
            return (t.reshape(t.shape[0] // 8, 8, n) * r_[None]).reshape(t.shape)

        def kproj(start, n):
            return jax.lax.dot_general(wt_v[pl.ds(D, D), :], x_v[rows(start, n), :], NT, preferred_element_type=f32)

        def sk(kt, off, r_):
            n = kt.shape[1]
            for g in range(HG):
                for s0 in range(0, n, SB):
                    phik_v[g, :, off + s0:off + s0 + SB] = _dual_softmax_hg(scale_rows(kt[g * 64:(g + 1) * 64, s0:s0 + SB], r_[:, s0:s0 + SB]))

        def vproj(start, n, off, r_):
            vt = jax.lax.dot_general(wt_v[pl.ds(2 * D, D), :], x_v[rows(start, n), :], NT, preferred_element_type=f32)
            for g in range(HG):
                v_v[g, 0:64, off:off + n] = scale_rows(vt[g * 64:(g + 1) * 64], r_).astype(bf16)

        def kvacc(first):
            for g in range(HG):
                t = jax.lax.dot_general(v_v[g], phik_v[g], NT, preferred_element_type=f32)
                if first:
                    acc_v[g] = t
                else:
                    acc_v[g] += t

        with scope("s01_prepk"):
            cp['wk'].wait()
            prep(1, pts, LOG2E)
        issue(1)
        with scope("s1_first"):
            cp['x0'].wait()
            ra = rstd(0, CA, 0)
            kta = kproj(0, CA)
            issue(21)
            cp['wv'].wait()
            prep(2, [perm] * G, None)
            cp['x1'].wait()
            issue(22)
            rb = rstd(CA, CA, CA)
            vproj(0, CA, 0, ra)
            sk(kta, 0, ra)
            ktb = kproj(CA, CA)
            vproj(CA, CA, CA, rb)
            sk(ktb, CA, rb)
            kvacc(True)
        issue(2)
        with scope("s3_p1loop"):
            cp['x2'].wait()
            for ci in range(1, n1):
                issue(10 + ci)
                r_ = rstd(ci * C1, C1, 0)
                kt = kproj(ci * C1, C1)
                vproj(ci * C1, C1, 0, r_)
                sk(kt, 0, r_)
                kvacc(False)
        issue(3)

        def qproj(ci):
            return jax.lax.dot_general(wt_v[pl.ds(0, D), :], x_v[rows2(ci), :], NT, preferred_element_type=f32)

        def sq(ci, pq):
            r_ = rt_v[:, pl.ds(pl.multiple_of(ci * C2, C2), C2)]
            for g in range(HG):
                for s0 in range(0, C2, SB):
                    phiq_v[g, :, s0:s0 + SB] = _dual_softmax_hg(scale_rows(pq[g * 64:(g + 1) * 64, s0:s0 + SB], r_[:, s0:s0 + SB]))

        def num():
            for g in range(HG):
                nd = jnp.dot(kvz_v[g], phiq_v[g], preferred_element_type=f32)
                if MR > 64:
                    rden = 1.0 / (nd[64:72] + 1e-6)
                    o = (nd[:64].reshape(8, 8, C2) * rden[None]).reshape(64, C2)
                else:
                    o = nd * 0.001
                ot_v[pl.ds(g * 64, 64), :] = o.astype(bf16)

        def wo_ln(ci):
            attn = jax.lax.dot_general(ot_v[...], wop_v[...], TN, preferred_element_type=f32)
            b2 = b2_ref[...].astype(f32).reshape(1, D)
            for b in range(0, C2, RB):
                r_ = rows2(ci, b, RB)
                h = x_v[r_, :].astype(f32) + attn[b:b + RB]
                h_v[r_, :] = h + b2
                hn_v[r_, :] = _ln(h, lnpos).astype(bf16)

        def m1(ci):
            a = jnp.dot(hn_v[rows2(ci), :], w1_v[...], preferred_element_type=f32)
            a = a + b1_ref[...].astype(f32).reshape(1, F)
            a = jnp.maximum(a, 0.0)
            return (a * a).astype(bf16)

        def ocopy(ci):
            return pltpu.make_async_copy(out_v.at[rows2(ci)], out_hbm.at[rows2(ci)], sem_o.at[ci])

        def m2(ci, a):
            o = jnp.dot(a, w2_v[...], preferred_element_type=f32) + h_v[rows2(ci), :]
            out_v[rows2(ci), :] = o.astype(bf16)
            ocopy(ci).start()

        with scope("s4_trans"):
            cp['wq'].wait()
            prep(0, pts, LOG2E)
            pq0 = qproj(0)
            pq1 = qproj(1)
            sq(0, pq0)
            rr = jax.lax.broadcasted_iota(jnp.int32, (MR, 128), 0)
            cc = jax.lax.broadcasted_iota(jnp.int32, (MR, 128), 1)
            hm = (rr % 4) == (cc % 4)
            for g in range(HG):
                a_ = acc_v[g]
                kv = a_[0:64] - (cs_v[pl.ds(g * 64, 64), :].reshape(8, 8, 128) * a_[72:80][None]).reshape(64, 128)
                kvz_v[g] = jnp.where(hm, jnp.concatenate([kv, a_[64:80]], axis=0), 0.0).astype(bf16)
            num()
            cp['wo'].wait()
            cp['b2'].wait()
            for g in range(G):
                t = jnp.dot(perm, wo_v[pl.ds(g * 128, 128), :], preferred_element_type=f32)
                wop_v[pl.ds(g * 128, 128), :] = t.astype(bf16)
            if order == 0:
                wo_ln(0)
                sq(1, pq1)
            else:
                sq(1, pq1)
                wo_ln(0)
            num()
            cp['b1'].wait()
            cp['w1'].wait()
            cp['w2'].wait()

        def body(ci, do_w, do_q):
            if do_q:
                pq = qproj(ci + 2)
            a = m1(ci)
            if do_q and order == 1:
                sq(ci + 2, pq)
            if do_w:
                wo_ln(ci + 1)
            if do_q and order == 0:
                sq(ci + 2, pq)
            if do_q:
                num()
            m2(ci, a)

        with scope("s5_p2loop"):
            if unroll2:
                for ci in range(n2 - 2):
                    body(ci, True, True)
            else:
                @pl.loop(0, n2 - 2, unroll=unr)
                def _(ci):
                    body(ci, True, True)
        with scope("s6_p2last"):
            body(n2 - 2, True, False)
            ci = n2 - 1
            a = m1(ci)
            tb = C2 // tail_split
            cps = []
            for t in range(tail_split):
                r_ = rows2(ci, t * tb, tb)
                o = jnp.dot(a[t * tb:(t + 1) * tb], w2_v[...], preferred_element_type=f32) + h_v[r_, :]
                out_v[r_, :] = o.astype(bf16)
                cps.append(pltpu.make_async_copy(out_v.at[r_], out_hbm.at[r_], sem_o.at[n2 + t]))
                cps[-1].start()
        with scope("s7_tail"):
            for c in range(n2 - 1):
                ocopy(c).wait()
            for c_ in cps:
                c_.wait()

    return kernel, n2, C1


PLANS = {
    1: {0: ('wp', 'wk', 'x0'), 20: ('wv', 'x1'), 1: ('x2',), 21: ('wq', 'wo', 'b1', 'b2'), 22: ('w1', 'w2')},
    3: {0: ('wp', 'wk', 'x0', 'wv', 'x1'), 1: ('x2', 'wq', 'wo', 'b1', 'b2'), 22: ('w1', 'w2')},
    4: {0: ('wp', 'wk', 'x0', 'wv', 'x1'), 20: ('x2',), 1: ('wq', 'wo', 'b1', 'b2', 'w1', 'w2')},
}


def build(C2=256, RB=64, scopes=False, plan=4, tail_split=2, SB=256, MR=80, order=0, lnpos=0, unroll2=False, unr=1, flags=None):
    kernel, n2, C1 = make_kernel(C2, RB, scopes, tail_split, min(SB, C2), MR, order, PLANS[plan], lnpos, unroll2, unr)

    @jax.jit
    def fn(A_x, A_wqkv, A_w_phi, A_wo, B_x, B_w1, B_b1, B_w2, B_b2):
        del B_x
        anyspec = pl.BlockSpec(memory_space=pl.ANY)
        vspec = pl.BlockSpec(memory_space=pltpu.VMEM)
        out = pl.pallas_call(
            kernel,
            out_shape=jax.ShapeDtypeStruct((S, D), bf16),
            in_specs=[anyspec] * 8,
            out_specs=anyspec,
            scratch_shapes=[
                pltpu.VMEM((DH * DH, H), bf16),
                pltpu.VMEM((F,), bf16),
                pltpu.VMEM((D,), bf16),
                pltpu.VMEM((8, S), f32),
                pltpu.VMEM((D, 128), f32),
                pltpu.VMEM((S, D), bf16),
                pltpu.VMEM((3, D, D), bf16),
                pltpu.VMEM((3 * D, D), bf16),
                pltpu.VMEM((D, D), bf16),
                pltpu.VMEM((D, D), bf16),
                pltpu.VMEM((D, F), bf16),
                pltpu.VMEM((F, D), bf16),
                pltpu.VMEM((HG, MR, 128), f32),
                pltpu.VMEM((HG, MR, 128), bf16),
                pltpu.VMEM((S, D), bf16),
                pltpu.VMEM((S, D), f32),
                pltpu.VMEM((S, D), bf16),
                pltpu.VMEM((HG, 128, C1), bf16),
                pltpu.VMEM((HG, MR, C1), bf16),
                pltpu.VMEM((HG, 128, C2), bf16),
                pltpu.VMEM((D, C2), bf16),
                pltpu.SemaphoreType.DMA((8,)),
                pltpu.SemaphoreType.DMA((9,)),
                pltpu.SemaphoreType.DMA((n2 + 8,)),
            ],
            compiler_params=pltpu.CompilerParams(vmem_limit_bytes=100 * 2**20, flags=flags),
        )(A_x.reshape(S, D), A_wqkv, A_w_phi.transpose(1, 2, 0).reshape(DH * DH, H), A_wo, B_w1,
          B_b1, B_w2, B_b2)
        return out.reshape(A_x.shape)
    return fn


pallas_sequential_preLN__linear_kernel_hedgehog__dense_activation_squared_relu__prompt_kernel = build(plan=4, lnpos=1, unr=2)
```

```python
import jax
import jax.numpy as jnp
import numpy as np
import jax.experimental.pallas as pl
import jax.experimental.pallas.tpu as pltpu

S, D, H, DH, F = 2048, 512, 32, 16, 1792
G = 4
HG = 8
C1 = 512
C2 = 256
KA = 256
RB = 128
WS = 128
TS = 4
N1, N2 = S // C1, S // C2
LOG2E = float(np.log2(np.e))
NT = (((1,), (1,)), ((), ()))
TN = (((0,), (0,)), ((), ()))
f32, bf16 = jnp.float32, jnp.bfloat16


def _ln(x):
    m = jnp.sum(x, axis=-1, keepdims=True) * (1.0 / D)
    v = jnp.maximum(jnp.sum(x * x, axis=-1, keepdims=True) * (1.0 / D) - m * m, 0.0)
    return (x - m) * jax.lax.rsqrt(v + 1e-5)


def _red(op, fn, a):
    m = fn(a, axis=0)
    return op(m, pltpu.roll(m, 4, axis=0))[None]


def _dual_softmax(p, z=None):
    n = p.shape[-1]
    p3 = p.reshape(8, 8, n)
    ep = jnp.exp2(p3 - _red(jnp.maximum, jnp.max, p3))
    en = jnp.exp2(_red(jnp.minimum, jnp.min, p3) - p3)
    rp = 1.0 / _red(jnp.add, jnp.sum, ep)
    rn = 1.0 / _red(jnp.add, jnp.sum, en)
    if z is not None:
        zp, zn = z
        den = _red(jnp.add, jnp.sum, ep * zp) * rp + _red(jnp.add, jnp.sum, en * zn) * rn + 1e-6
        rd = 1.0 / den
        rp = rp * rd
        rn = rn * rd
    pp = (ep * rp).reshape(64, n)
    pn = (en * rn).reshape(64, n)
    return jnp.concatenate([pp, pn], axis=0).astype(bf16)


def _scale_rows(t, r):
    n = t.shape[1]
    return (t.reshape(t.shape[0] // 8, 8, n) * r[None]).reshape(t.shape)


def _iota(shape, dim):
    return jax.lax.broadcasted_iota(jnp.int32, shape, dim)


def _kernel(x_hbm, wqkv_hbm, wphi_hbm, wo_hbm, w1_hbm, b1_hbm, w2_hbm, b2_hbm, out_hbm,
            wphi_v, b1_v, b2_v, rt_v, cs_v, zb_v,
            x_v, wqkv_v, wt_v, wo_v, w1_v, w2_v, acc_v, kv_v, out_v, h_v, hn_v,
            phik_v, v_v, phiq_v, ot_v,
            sem_x, sem_w, sem_o):
    def rows2(ci, off=0, n=C2):
        return pl.ds(pl.multiple_of(ci * C2 + off, n), n)

    def wcopy(part, i):
        return pltpu.make_async_copy(wqkv_hbm.at[:, pl.ds(part * D, D)], wqkv_v.at[part], sem_w.at[i])

    def xcopy(start, n, i):
        return pltpu.make_async_copy(x_hbm.at[pl.ds(start, n)], x_v.at[pl.ds(start, n)], sem_x.at[i])

    cp = dict(wk=wcopy(1, 0), wv=wcopy(2, 1), wq=wcopy(0, 2),
              wo=pltpu.make_async_copy(wo_hbm, wo_v, sem_w.at[3]),
              w1=pltpu.make_async_copy(w1_hbm, w1_v, sem_w.at[4]),
              w2=pltpu.make_async_copy(w2_hbm, w2_v, sem_w.at[5]),
              wp=pltpu.make_async_copy(wphi_hbm, wphi_v, sem_w.at[6]),
              b1=pltpu.make_async_copy(b1_hbm, b1_v, sem_w.at[7]),
              b2=pltpu.make_async_copy(b2_hbm, b2_v, sem_w.at[8]),
              x0=xcopy(0, C1, 0), x1=xcopy(C1, S - C1, 1))
    for name in ('wp', 'wk', 'x0', 'wv'):
        cp[name].start()

    r, c = _iota((128, 128), 0), _iota((128, 128), 1)
    same_head = ((r // 64) * 4 + r % 4) == (c // 16)
    e = jnp.where(_iota((H, D), 0) == _iota((H, D), 1) // 16, 1.0, 0.0).astype(bf16)
    same_d = _iota((256, D), 0) // 16 == _iota((256, D), 1) % 16
    r3 = jnp.where((_iota((128, 256), 0) % 64) // 4 == _iota((128, 256), 1) % 16, 1.0, 0.0).astype(bf16)
    cp['wp'].wait()
    cp['x1'].start()
    a = jnp.where(same_d, jnp.dot(wphi_v[...], e, preferred_element_type=f32), 0.0).astype(bf16)
    pts = []
    for g in range(G):
        t = jnp.dot(r3, a[:, g * 128:(g + 1) * 128], preferred_element_type=f32)
        pts.append(jnp.where(same_head, t, 0.0).astype(bf16))

    def prep(part):
        for g in range(G):
            w = wqkv_v[part, :, pl.ds(g * 128, 128)]
            t = jax.lax.dot_general(pts[g], w, NT, preferred_element_type=f32)
            t = (t - jnp.sum(t, axis=1, keepdims=True) * (1.0 / D)) * LOG2E
            wt_v[pl.ds(part * D + g * 128, 128), :] = t.astype(bf16)

    def prepv():
        for g in range(G):
            t = wqkv_v[2, :, pl.ds(g * 128, 128)].T
            wt_v[pl.ds(2 * D + g * 128, 128), :] = t
            cs = jnp.sum(t.astype(f32), axis=1, keepdims=True)
            cs_v[pl.ds(g * 128, 128), :] = jnp.broadcast_to(cs, (128, 128))

    def stats(start, n):
        def red(t):
            t = jnp.sum(t.T.reshape(16, 8, 128), axis=0)
            t = t + pltpu.roll(t, 4, axis=0)
            t = t + pltpu.roll(t, 2, axis=0)
            return t + pltpu.roll(t, 1, axis=0)
        rs, ms = [], []
        for b in range(0, n, 128):
            xf = x_v[pl.ds(start + b, 128), :].astype(f32)
            s1 = xf[:, 0:128]
            s2 = s1 * s1
            for t in range(1, D // 128):
                xt = xf[:, t * 128:(t + 1) * 128]
                s1 = s1 + xt
                s2 = s2 + xt * xt
            m = red(s1) * (1.0 / D)
            v = jnp.maximum(red(s2) * (1.0 / D) - m * m, 0.0)
            rs.append(jax.lax.rsqrt(v + 1e-5))
            ms.append(m)
        return jnp.concatenate(rs, axis=1), jnp.concatenate(ms, axis=1)

    def store_stats(start, off, rstd, mean):
        n = rstd.shape[1]
        rt_v[:, pl.ds(start, n)] = rstd
        ext = jnp.concatenate([jnp.ones((8, n), f32), rstd * mean], axis=0).astype(bf16)
        for g in range(HG):
            v_v[g, 64:80, off:off + n] = ext

    def proj(part, start, n, lo=0, hi=D):
        return jax.lax.dot_general(wt_v[pl.ds(part * D + lo, hi - lo), :], x_v[pl.ds(start, n), :], NT,
                                   preferred_element_type=f32)

    def phi_k(kt, rstd, off=0):
        for g in range(HG):
            for s0 in range(0, kt.shape[1], 128):
                p = _scale_rows(kt[g * 64:(g + 1) * 64, s0:s0 + 128], rstd[:, off + s0:off + s0 + 128])
                phik_v[g, :, off + s0:off + s0 + 128] = _dual_softmax(p)

    def vproj(start, rstd):
        vt = proj(2, start, C1)
        for g in range(HG):
            v_v[g, 0:64, :] = _scale_rows(vt[g * 64:(g + 1) * 64], rstd).astype(bf16)

    def kvacc(first):
        for g in range(HG):
            t = jax.lax.dot_general(v_v[g], phik_v[g], NT, preferred_element_type=f32)
            if first:
                acc_v[g] = t
            else:
                acc_v[g] += t

    cp['wk'].wait()
    prep(1)
    for name in ('wq', 'wo', 'b1', 'b2', 'w1', 'w2'):
        cp[name].start()
    cp['x0'].wait()
    ra, ma = stats(0, KA)
    phi_k(proj(1, 0, KA), ra)
    cp['wv'].wait()
    store_stats(0, 0, ra, ma)
    rb, mb = stats(KA, C1 - KA)
    store_stats(KA, KA, rb, mb)
    r0 = jnp.concatenate([ra, rb], axis=1)
    prepv()
    ktb = proj(1, KA, C1 - KA)
    vproj(0, r0)
    phi_k(ktb, r0, KA)
    cp['x1'].wait()
    kvacc(True)
    for ci in range(1, N1):
        rc, mc = stats(ci * C1, C1)
        store_stats(ci * C1, 0, rc, mc)
        kt = proj(1, ci * C1, C1)
        vproj(ci * C1, rc)
        phi_k(kt, rc)
        if ci < N1 - 1:
            kvacc(False)

    def qproj(ci, lo=0, hi=D):
        return proj(0, pl.multiple_of(ci * C2, C2), C2, lo, hi)

    def phi_q(ci, pq, g0=0):
        rstd = rt_v[:, pl.ds(pl.multiple_of(ci * C2, C2), C2)]
        for g in range(pq.shape[0] // 64):
            zt = zb_v[g0 + g]
            z = (zt[0:64].reshape(8, 8, 128), zt[64:128].reshape(8, 8, 128))
            for s0 in range(0, C2, 128):
                p = _scale_rows(pq[g * 64:(g + 1) * 64, s0:s0 + 128], rstd[:, s0:s0 + 128])
                phiq_v[g0 + g, :, s0:s0 + 128] = _dual_softmax(p, z)

    def num():
        for g in range(HG):
            o = jnp.dot(kv_v[g], phiq_v[g], preferred_element_type=f32)
            ot_v[pl.ds(g * 64, 64), :] = o.astype(bf16)

    def wo_ln(ci):
        b2 = b2_v[...].astype(f32).reshape(1, D)
        for b in range(0, C2, RB):
            if b % WS == 0:
                attn = jax.lax.dot_general(ot_v[:, b:b + WS], wo_v[...], TN, preferred_element_type=f32)
            rows = rows2(ci, b, RB)
            h = x_v[rows, :].astype(f32) + attn[b % WS:b % WS + RB]
            h_v[rows, :] = h + b2
            hn_v[rows, :] = _ln(h).astype(bf16)

    def m1(ci):
        t = jnp.dot(hn_v[rows2(ci), :], w1_v[...], preferred_element_type=f32)
        t = jnp.maximum(t + b1_v[...].astype(f32).reshape(1, F), 0.0)
        return (t * t).astype(bf16)

    def ocopy(ci, t, n, sem):
        rows = rows2(ci, t * n, n)
        return pltpu.make_async_copy(out_v.at[rows], out_hbm.at[rows], sem_o.at[sem])

    def m2(ci, act, t, n, sem):
        rows = rows2(ci, t * n, n)
        o = jnp.dot(act[t * n:(t + 1) * n], w2_v[...], preferred_element_type=f32) + h_v[rows, :]
        out_v[rows, :] = o.astype(bf16)
        ocopy(ci, t, n, sem).start()

    for name in ('wq', 'wo', 'b1', 'b2', 'w1', 'w2'):
        cp[name].wait()
    prep(0)
    kvacc(False)
    pq0 = qproj(0)
    pq1a = qproj(1, 0, D // 2)
    head = (_iota((64, 128), 0) // 16) == (_iota((64, 128), 1) % 4)
    for g in range(HG):
        t = acc_v[g]
        kv = t[0:64] - _scale_rows(cs_v[pl.ds(g * 64, 64), :], t[72:80])
        kv_v[g] = jnp.where(head, kv, 0.0).astype(bf16)
        zb_v[g] = jnp.broadcast_to(t[64:72][None], (16, 8, 128)).reshape(128, 128).T
    phi_q(0, pq0)
    num()
    pq1b = qproj(1, D // 2, D)
    wo_ln(0)
    phi_q(1, pq1a, 0)
    phi_q(1, pq1b, HG // 2)
    num()

    def body(ci, do_q):
        act = m1(ci)
        if do_q:
            pq = qproj(ci + 2)
        wo_ln(ci + 1)
        if do_q:
            phi_q(ci + 2, pq)
            num()
        m2(ci, act, 0, C2, ci)

    @pl.loop(0, N2 - 2)
    def _(ci):
        body(ci, True)

    body(N2 - 2, False)
    act = m1(N2 - 1)
    for t in range(TS):
        m2(N2 - 1, act, t, C2 // TS, N2 + t)
    for ci in range(N2 - 1):
        ocopy(ci, 0, C2, ci).wait()
    for t in range(TS):
        ocopy(N2 - 1, t, C2 // TS, N2 + t).wait()


@jax.jit
def pallas_sequential_preLN__linear_kernel_hedgehog__dense_activation_squared_relu__prompt_kernel(
    A_x: jax.Array,
    A_wqkv: jax.Array,
    A_w_phi: jax.Array,
    A_wo: jax.Array,
    B_x: jax.Array,
    B_w1: jax.Array,
    B_b1: jax.Array,
    B_w2: jax.Array,
    B_b2: jax.Array,
):
    del B_x
    anyspec = pl.BlockSpec(memory_space=pl.ANY)
    out = pl.pallas_call(
        _kernel,
        out_shape=jax.ShapeDtypeStruct((S, D), bf16),
        in_specs=[anyspec] * 8,
        out_specs=anyspec,
        scratch_shapes=[
            pltpu.VMEM((DH * DH, H), bf16),
            pltpu.VMEM((F,), bf16),
            pltpu.VMEM((D,), bf16),
            pltpu.VMEM((8, S), f32),
            pltpu.VMEM((D, 128), f32),
            pltpu.VMEM((HG, 128, 128), f32),
            pltpu.VMEM((S, D), bf16),
            pltpu.VMEM((3, D, D), bf16),
            pltpu.VMEM((3 * D, D), bf16),
            pltpu.VMEM((D, D), bf16),
            pltpu.VMEM((D, F), bf16),
            pltpu.VMEM((F, D), bf16),
            pltpu.VMEM((HG, 80, 128), f32),
            pltpu.VMEM((HG, 64, 128), bf16),
            pltpu.VMEM((S, D), bf16),
            pltpu.VMEM((S, D), f32),
            pltpu.VMEM((S, D), bf16),
            pltpu.VMEM((HG, 128, C1), bf16),
            pltpu.VMEM((HG, 80, C1), bf16),
            pltpu.VMEM((HG, 128, C2), bf16),
            pltpu.VMEM((D, C2), bf16),
            pltpu.SemaphoreType.DMA((2,)),
            pltpu.SemaphoreType.DMA((9,)),
            pltpu.SemaphoreType.DMA((N2 + TS,)),
        ],
        compiler_params=pltpu.CompilerParams(vmem_limit_bytes=100 * 2**20),
    )(A_x.reshape(S, D), A_wqkv, A_w_phi.transpose(1, 2, 0).reshape(DH * DH, H), A_wo,
      B_w1, B_b1, B_w2, B_b2)
    return out.reshape(A_x.shape)
```
